```python
import jax
import jax.numpy as jnp

def _softmax(x, axis=-1):
    return jax.nn.softmax(x, axis=axis)
def _gelu(x):
    return jax.nn.gelu(x, approximate=True)
def _silu(x):
    return jax.nn.silu(x)
def _sigmoid(x):
    return jax.nn.sigmoid(x)
def _layernorm(x, axis=-1, eps=1e-5):
    m = jnp.mean(x, axis=axis, keepdims=True)
    v = jnp.var(x, axis=axis, keepdims=True)
    return (x - m) / jnp.sqrt(v + eps)
def _scatter_add(tgt, idx, src, axis=0):
    return tgt.at[idx].add(src)
def _segment_sum(src, seg, n):
    return jax.ops.segment_sum(src, seg, n)
class _Rng:
    def __init__(self, key):
        self._k = key
    def _next(self):
        self._k, sub = jax.random.split(self._k)
        return sub
    def normal(self, shape):
        return jax.random.normal(self._next(), shape, dtype=jnp.bfloat16)
    def randint(self, lo, hi, shape):
        return jax.random.randint(self._next(), shape, lo, hi, dtype=jnp.int32)
    def uniform(self, shape, lo=0.0, hi=1.0):
        return jax.random.uniform(self._next(), shape, jnp.bfloat16, lo, hi)
    def permutation(self, n):
        return jax.random.permutation(self._next(), n)


kernel_name = 'sequential_preLN__linear_attn_block__moe_arch_mod__prompt'

def setup_inputs():
    _rng = _Rng(jax.random.key(int.from_bytes(__import__("os").urandom(4), "little")))
    _w = (lambda a: (lambda t: t.astype(jnp.bfloat16) if jnp.issubdtype(t.dtype, jnp.floating) else t)(jnp.asarray(a)))
    def _A_setup():
        B, S, D = 1, 2048, 1024
        return {
            "x": _w((lambda *s: _rng.normal(s) * 0.05)(B, S, D)),
            "wqkv": _w((lambda *s: _rng.normal(s) * 0.05)(D, 3 * D)),
            "wo": _w((lambda *s: _rng.normal(s) * 0.05)(D, D)),
        }
    _A_in = _A_setup()

    def _B_setup():
        B, S, D, F, C = 1, 2048, 1024, 3584, 2
        return {
            "x": _w((lambda *s: _rng.normal(s) * 0.05)(B, S, D)),
            "w_r": _w((lambda *s: _rng.normal(s) * 0.05)(D)),
            "w_gate": _w((lambda *s: _rng.normal(s) * 0.05)(D, F)),
            "w_up": _w((lambda *s: _rng.normal(s) * 0.05)(D, F)),
            "w_down": _w((lambda *s: _rng.normal(s) * 0.05)(F, D)),
        }
    _B_in = _B_setup()

    return {
        "A_x": _A_in["x"],
        "A_wqkv": _A_in["wqkv"],
        "A_wo": _A_in["wo"],
        "B_x": _B_in["x"],
        "B_w_r": _B_in["w_r"],
        "B_w_gate": _B_in["w_gate"],
        "B_w_up": _B_in["w_up"],
        "B_w_down": _B_in["w_down"],
    }

def reference(A_x, A_wqkv, A_wo, B_x, B_w_r, B_w_gate, B_w_up, B_w_down):
    def _A_ref(x, wqkv, wo):
        B, S, D = x.shape
        H = 32; Dh = D // H
        qkv = (lambda x, *d: x.transpose(*d))((x @ wqkv).reshape(B, S, 3, H, Dh), 2, 0, 3, 1, 4)
        q, k, v = qkv[0], qkv[1], qkv[2]
        phi = lambda t: jnp.where(t > 0, t + 1, jnp.exp(t)) + 1e-6
        pq, pk = phi(q), phi(k)
        kv = jnp.einsum("bhsd,bhse->bhde", pk, v)
        z = jnp.einsum("bhsd->bhd", pk)
        num = jnp.einsum("bhqd,bhde->bhqe", pq, kv)
        den = jnp.einsum("bhqd,bhd->bhq", pq, z)[..., None] + 1e-6
        o = num / den
        return (lambda x, *d: x.transpose(*d))(o, 0, 2, 1, 3).reshape(B, S, D) @ wo

    def _B_ref(x, w_r, w_gate, w_up, w_down):
        B, S, D = x.shape
        C = 2
        r = x @ w_r
        idx = jnp.argsort(-r, axis=-1)[:, :C]
        idx_e = jnp.repeat(idx.reshape(B, C, 1), D, axis=2)
        x_sel = jnp.take_along_axis(x, idx_e, axis=1)
        g = _silu(x_sel @ w_gate)
        u = x_sel @ w_up
        y = (g * u) @ w_down
        r_sel = _sigmoid(jnp.take_along_axis(r, idx, axis=1))
        y = y * r_sel.reshape(B, C, 1)
        b_off = (jnp.arange(B) * S).reshape(B, 1)
        flat_idx = (idx + b_off).reshape(B * C)
        zero = (x * 0.0).reshape(B * S, D)
        upd = _scatter_add(zero, flat_idx, y.reshape(B * C, D), axis=0)
        return x + upd.reshape(B, S, D)

    x = A_x
    h = x + _A_ref(_layernorm(x, axis=-1), A_wqkv, A_wo)
    h2 = h + _B_ref(_layernorm(h, axis=-1), B_w_r, B_w_gate, B_w_up, B_w_down)
    return h2
```

```python
import functools
import jax
import jax.numpy as jnp
import jax.experimental.pallas as pl
import jax.experimental.pallas.tpu as pltpu

S, D, F, DH = 2048, 1024, 3584, 32
G = D // 128
TM = 256
NB = S // TM
f32, bf16 = jnp.float32, jnp.bfloat16
NT = (((1,), (1,)), ((), ()))


def _phi(t):
    return jnp.where(t > 0, t + 1.0, jnp.exp(t)) + 1e-6


def _ln(x):
    m = jnp.mean(x, axis=-1, keepdims=True)
    xc = x - m
    v = jnp.mean(xc * xc, axis=-1, keepdims=True)
    return xc * jax.lax.rsqrt(v + 1e-5)


def _dot(a, b):
    return jnp.dot(a, b, preferred_element_type=f32)


def _kernel(x_hbm, wqkv_hbm, wo_hbm, wr_ref, wg_hbm, wu_hbm, wd_hbm, out_hbm,
            x_v, wq_v, wk_v, wv_v, wkT_v, wo_v, wg_v, wu_v, wd_v, pq_v, ln2_v, out_v,
            m_v, zb_v, kv_v, z_v, top_v, topi_v, xsem, wsem, osem, psem):
    def x_copy(i):
        return pltpu.make_async_copy(x_hbm.at[pl.ds(i * TM, TM)], x_v.at[pl.ds(i * TM, TM)], xsem.at[i])

    def o_copy(i):
        return pltpu.make_async_copy(out_v.at[pl.ds(i * TM, TM)], out_hbm.at[pl.ds(i * TM, TM)], osem.at[i])

    c_wq = pltpu.make_async_copy(wqkv_hbm.at[:, pl.ds(0, D)], wq_v, wsem.at[0])
    c_wk = pltpu.make_async_copy(wqkv_hbm.at[:, pl.ds(D, D)], wk_v, wsem.at[1])
    c_wv = pltpu.make_async_copy(wqkv_hbm.at[:, pl.ds(2 * D, D)], wv_v, wsem.at[2])
    c_wo = pltpu.make_async_copy(wo_hbm, wo_v, wsem.at[3])
    c_wg = pltpu.make_async_copy(wg_hbm, wg_v, wsem.at[4])
    c_wu = pltpu.make_async_copy(wu_hbm, wu_v, wsem.at[5])
    c_wd = pltpu.make_async_copy(wd_hbm, wd_v, wsem.at[6])

    x_copy(0).start()
    c_wk.start()
    c_wq.start()
    c_wv.start()
    for i in range(1, NB):
        x_copy(i).start()
    c_wo.start()
    c_wk.wait()
    wkT_v[...] = wk_v[...].T
    c_wq.wait()
    c_wv.wait()
    c_wg.start()
    c_wu.start()
    c_wd.start()

    kv_v[...] = jnp.zeros_like(kv_v)
    z_v[...] = jnp.zeros_like(z_v)

    def p1(i, _):
        r0 = pl.multiple_of(i * TM, TM)
        x_copy(i).wait()
        ln = _ln(x_v[pl.ds(r0, TM), :].astype(f32)).astype(bf16)
        q = _dot(ln, wq_v[...])
        pq_v[pl.ds(r0, TM), :] = _phi(q).astype(bf16)
        pkT = _phi(jax.lax.dot_general(wkT_v[...], ln, NT, preferred_element_type=f32))
        zs = pkT[:, 0:128]
        for c in range(1, TM // 128):
            zs = zs + pkT[:, c * 128:(c + 1) * 128]
        z_v[...] += zs
        pkT = pkT.astype(bf16)
        v = _dot(ln, wv_v[...]).astype(bf16)
        for g in range(G):
            sl = slice(g * 128, (g + 1) * 128)
            kv_v[sl, :] += _dot(pkT[sl, :], v[:, sl])
        return 0

    jax.lax.fori_loop(0, NB, p1, 0)

    c_wo.wait()
    ri = jax.lax.broadcasted_iota(jnp.int32, (128, 128), 0) // DH
    ci = jax.lax.broadcasted_iota(jnp.int32, (128, 128), 1) // DH
    msk = ri == ci
    for g in range(G):
        sl = slice(g * 128, (g + 1) * 128)
        zc = jnp.sum(z_v[sl, :], axis=-1, keepdims=True)
        zb_v[sl, :] = jnp.where(msk, zc, 0.0).astype(bf16)
        kvm = jnp.where(msk, kv_v[sl, :], 0.0).astype(bf16)
        m_v[sl, :] = _dot(kvm, wo_v[sl, :]).astype(bf16)

    top_v[...] = jnp.full(top_v.shape, -jnp.inf, f32)
    topi_v[...] = jnp.zeros(topi_v.shape, jnp.int32)
    wr = wr_ref[...].astype(f32)
    BIG = 1 << 20

    def p2(i, _):
        r0 = pl.multiple_of(i * TM, TM)
        parts = []
        for g in range(G):
            sl = slice(g * 128, (g + 1) * 128)
            pq = pq_v[pl.ds(r0, TM), sl]
            den = _dot(pq, zb_v[sl, :]) + 1e-6
            parts.append((pq.astype(f32) / den).astype(bf16))
        pqn = jnp.concatenate(parts, axis=1)
        h = x_v[pl.ds(r0, TM), :].astype(f32) + _dot(pqn, m_v[...])
        ln2 = _ln(h)
        out_v[pl.ds(r0, TM), :] = (h + ln2).astype(bf16)
        o_copy(i).start()
        ln2_v[pl.ds(r0, TM), :] = ln2.astype(bf16)
        r = jnp.sum(ln2 * wr, axis=-1, keepdims=True)
        ids = jax.lax.broadcasted_iota(jnp.int32, (TM, 1), 0) + r0
        m1 = jnp.max(r, axis=0, keepdims=True)
        i1 = jnp.min(jnp.where(r == m1, ids, BIG), axis=0, keepdims=True)
        r2 = jnp.where(ids == i1, -jnp.inf, r)
        m2 = jnp.max(r2, axis=0, keepdims=True)
        i2 = jnp.min(jnp.where((r2 == m2) & (ids != i1), ids, BIG), axis=0, keepdims=True)
        b1, b2 = top_v[0:1, :], top_v[1:2, :]
        j1, j2 = topi_v[0:1, :], topi_v[1:2, :]
        new_first = m1 > b1
        n1 = jnp.where(new_first, m1, b1)
        k1 = jnp.where(new_first, i1, j1)
        ca = jnp.where(new_first, b1, m1)
        ka = jnp.where(new_first, j1, i1)
        cb = jnp.where(new_first, m2, b2)
        kb = jnp.where(new_first, i2, j2)
        take_b = cb > ca
        n2 = jnp.where(take_b, cb, ca)
        k2 = jnp.where(take_b, kb, ka)
        top_v[0:1, :] = jnp.broadcast_to(n1, (1, 128))
        top_v[1:2, :] = jnp.broadcast_to(n2, (1, 128))
        topi_v[0:1, :] = jnp.broadcast_to(k1, (1, 128))
        topi_v[1:2, :] = jnp.broadcast_to(k2, (1, 128))
        return 0

    jax.lax.fori_loop(0, NB, p2, 0)

    idv = topi_v[...]
    idx = [idv[0, 0], idv[1, 0]]
    rsel = jax.nn.sigmoid(top_v[...][0:2, 0:1])
    rows16 = jax.lax.broadcasted_iota(jnp.int32, (16, D), 0)
    xs = jnp.zeros((16, D), f32)
    bases = []
    for c in range(2):
        base = pl.multiple_of((idx[c] // 16) * 16, 16)
        bases.append(base)
        t = ln2_v[pl.ds(base, 16), :].astype(f32)
        row = jnp.sum(jnp.where(rows16 == idx[c] % 16, t, 0.0), axis=0, keepdims=True)
        xs = jnp.where(rows16 == c, row, xs)
    xs = xs.astype(bf16)
    c_wg.wait()
    gte = _dot(xs, wg_v[...])
    c_wu.wait()
    up = _dot(xs, wu_v[...])
    a = (jax.nn.silu(gte) * up).astype(bf16)
    c_wd.wait()
    y = _dot(a, wd_v[...])
    y2 = y[0:2, :] * rsel
    for i in range(NB):
        o_copy(i).wait()
    for c in range(2):
        t = out_v[pl.ds(bases[c], 16), :].astype(f32)
        t = jnp.where(rows16 == idx[c] % 16, t + y2[c:c + 1, :], t)
        out_v[pl.ds(bases[c], 16), :] = t.astype(bf16)

    def p_copy(c):
        return pltpu.make_async_copy(out_v.at[pl.ds(bases[c], 16)], out_hbm.at[pl.ds(bases[c], 16)], psem.at[c])

    p_copy(0).start()

    @pl.when(bases[0] != bases[1])
    def _():
        p_copy(1).start()
        p_copy(1).wait()

    p_copy(0).wait()


@jax.jit
def pallas_sequential_preLN__linear_attn_block__moe_arch_mod__prompt_kernel(
        A_x, A_wqkv, A_wo, B_x, B_w_r, B_w_gate, B_w_up, B_w_down):
    any_spec = pl.BlockSpec(memory_space=pl.ANY)
    out = pl.pallas_call(
        _kernel,
        in_specs=[any_spec, any_spec, any_spec, pl.BlockSpec(memory_space=pltpu.VMEM), any_spec, any_spec, any_spec],
        out_specs=any_spec,
        out_shape=jax.ShapeDtypeStruct((S, D), bf16),
        scratch_shapes=[
            pltpu.VMEM((S, D), bf16), pltpu.VMEM((D, D), bf16), pltpu.VMEM((D, D), bf16), pltpu.VMEM((D, D), bf16),
            pltpu.VMEM((D, D), bf16), pltpu.VMEM((D, D), bf16),
            pltpu.VMEM((D, F), bf16), pltpu.VMEM((D, F), bf16), pltpu.VMEM((F, D), bf16),
            pltpu.VMEM((S, D), bf16), pltpu.VMEM((S, D), bf16), pltpu.VMEM((S, D), bf16),
            pltpu.VMEM((D, D), bf16), pltpu.VMEM((D, 128), bf16), pltpu.VMEM((D, 128), f32), pltpu.VMEM((D, 128), f32),
            pltpu.VMEM((8, 128), f32), pltpu.VMEM((8, 128), jnp.int32),
            pltpu.SemaphoreType.DMA((NB,)), pltpu.SemaphoreType.DMA((7,)), pltpu.SemaphoreType.DMA((NB,)),
            pltpu.SemaphoreType.DMA((2,)),
        ],
        compiler_params=pltpu.CompilerParams(vmem_limit_bytes=100 * 1024 * 1024),
    )(A_x.reshape(S, D), A_wqkv, A_wo, B_w_r.reshape(1, D), B_w_gate, B_w_up, B_w_down)
    return out.reshape(1, S, D)
```

```python
import jax
import jax.numpy as jnp
import jax.experimental.pallas as pl
import jax.experimental.pallas.tpu as pltpu

S, D, F, DH = 2048, 1024, 3584, 32
G = D // 128
TM = 512
NB = S // TM
HD = 128
TM2 = 1024
SB2 = 256
NB2 = S // TM2
NC = 4
CW = D // NC
NC2 = 4
CW2 = D // NC2
RP = 0
NW = 1024
ORD = 'bac'
CS = 1
f32, bf16 = jnp.float32, jnp.bfloat16
NT = (((1,), (1,)), ((), ()))


def _phi(t):
    return jnp.where(t > 0, t + 1.0, jnp.exp(t)) + 1e-6


def _ln(x):
    m = jnp.mean(x, axis=-1, keepdims=True)
    xc = x - m
    v = jnp.mean(xc * xc, axis=-1, keepdims=True)
    return xc * jax.lax.rsqrt(v + 1e-5)


def _dot(a, b):
    return jnp.dot(a, b, preferred_element_type=f32)


def _dot_nt(a, b):
    return jax.lax.dot_general(a, b, NT, preferred_element_type=f32)


def _kernel(x_hbm, wqkv_hbm, wo_hbm, wr_ref, wg_hbm, wu_hbm, wd_hbm, out_hbm,
            x_v, wq_v, wk_v, wv_v, wkT_v, wo_v, wg_v, wu_v, wd_v, pq_v, ln2_v, out_v,
            m_v, zb_v, kv_v, z_v, lnc_v, r_v, h_v, xsem, wsem, osem, psem):
    def x_copy(i):
        return pltpu.make_async_copy(x_hbm.at[pl.ds(i * TM, TM)], x_v.at[pl.ds(i * TM, TM)], xsem.at[i])

    def o_copy(i):
        return pltpu.make_async_copy(out_v.at[pl.ds(i * SB2, SB2)], out_hbm.at[pl.ds(i * SB2, SB2)], osem.at[i])

    def wq_copy(c):
        return pltpu.make_async_copy(wqkv_hbm.at[:, pl.ds(c * CW, CW)], wq_v.at[:, pl.ds(c * CW, CW)], wsem.at[6 + c])

    c_wk = pltpu.make_async_copy(wqkv_hbm.at[:, pl.ds(D, D)], wk_v, wsem.at[0])
    c_wv = pltpu.make_async_copy(wqkv_hbm.at[:, pl.ds(2 * D, D)], wv_v, wsem.at[1])
    c_wo = pltpu.make_async_copy(wo_hbm, wo_v, wsem.at[2])
    c_wg = pltpu.make_async_copy(wg_hbm, wg_v, wsem.at[3])
    c_wu = pltpu.make_async_copy(wu_hbm, wu_v, wsem.at[4])
    c_wd = pltpu.make_async_copy(wd_hbm, wd_v, wsem.at[5])

    x_copy(0).start()
    for c in range(NC):
        wq_copy(c).start()

    kv_v[...] = jnp.zeros_like(kv_v)
    z_v[...] = jnp.zeros_like(z_v)

    def ln_rows(r, n):
        return _ln(x_v[pl.ds(r, n), :].astype(f32)).astype(bf16)

    def p1(i, first):
        r0 = pl.multiple_of(i * TM, TM)
        if first:
            x_copy(0).wait()
            ln = ln_rows(0, TM)
            for c in range(NC):
                cs = slice(c * CW, (c + 1) * CW)
                wq_copy(c).wait()
                if c == 0:
                    c_wv.start()
                if c == 2:
                    c_wk.start()
                pq_v[0:TM, cs] = _phi(_dot(ln, wq_v[:, cs])).astype(bf16)
            c_wv.wait()
            x_copy(1).start()
        else:
            head = lnc_v[...]
            RS = (TM - HD) // NC
            rest = []
            for c in range(NC):
                cs = slice(c * CW, (c + 1) * CW)
                pq_v[pl.ds(r0, HD), cs] = _phi(_dot(head, wq_v[:, cs])).astype(bf16)
                rest.append(ln_rows(r0 + HD + c * RS, RS))
            rest = jnp.concatenate(rest, axis=0)
            for c in range(NC):
                cs = slice(c * CW, (c + 1) * CW)
                pq_v[pl.ds(r0 + HD, TM - HD), cs] = _phi(_dot(rest, wq_v[:, cs])).astype(bf16)
            ln = jnp.concatenate([head, rest], axis=0)
        nxt = pl.multiple_of(jnp.minimum(r0 + TM, S - TM), TM)
        vs = []
        for c in range(NC):
            cs = slice(c * CW, (c + 1) * CW)
            vs.append(_dot(ln, wv_v[:, cs]).astype(bf16))
            if first and c == 1:
                c_wk.wait()
                for j in range(2, NB):
                    x_copy(j).start()
                c_wo.start()
            if first and c >= 1:
                for t in ((0, 1), (2,), (3,))[c - 1]:
                    ts = slice(t * CW, (t + 1) * CW)
                    wkT_v[ts, :] = wk_v[:, ts].T
        HS = HD // NC
        if first:
            x_copy(1).wait()
            c_wg.start()
            c_wu.start()
            c_wd.start()
        for c in range(NC):
            cs = slice(c * CW, (c + 1) * CW)
            pkT = _phi(_dot_nt(wkT_v[cs, :], ln))
            zs = pkT[:, 0:128]
            for t in range(1, TM // 128):
                zs = zs + pkT[:, t * 128:(t + 1) * 128]
            z_v[cs, :] += zs
            pkT = pkT.astype(bf16)
            for g in range(CW // 128):
                sl = slice(g * 128, (g + 1) * 128)
                kv_v[c * CW + g * 128:c * CW + (g + 1) * 128, :] += _dot(pkT[sl, :], vs[c][:, sl])
            lnc_v[c * HS:(c + 1) * HS, :] = ln_rows(nxt + c * HS, HS)

    p1(0, True)

    def p1_loop(i, _):
        @pl.when(i + 1 < NB)
        def _():
            x_copy(i + 1).wait()
        p1(i, False)

    jax.lax.fori_loop(1, NB, p1_loop, None)

    c_wo.wait()
    ri = jax.lax.broadcasted_iota(jnp.int32, (128, 128), 0) // DH
    ci = jax.lax.broadcasted_iota(jnp.int32, (128, 128), 1) // DH
    msk = ri == ci
    for g in range(G):
        sl = slice(g * 128, (g + 1) * 128)
        zc = jnp.sum(z_v[sl, :], axis=-1, keepdims=True)
        zb_v[sl, :] = jnp.where(msk, zc, 0.0).astype(bf16)
        kvm = jnp.where(msk, kv_v[sl, :], 0.0).astype(bf16)
        m_v[sl, :] = _dot(kvm, wo_v[sl, :]).astype(bf16)

    wr = jnp.broadcast_to(wr_ref[...].reshape(1, D), (16, D))

    def p2(i, _):
        r0 = pl.multiple_of(i * TM2, TM2)
        ns = TM2 // SB2
        RC = SB2 // NC2 // CS

        def stage_a(s, g):
            sl = slice(g * 128, (g + 1) * 128)
            pq = pq_v[pl.ds(r0 + s * SB2, SB2), sl]
            den = _dot(pq, zb_v[sl, :]) + 1e-6
            rc = pl.reciprocal(den, approx=True)
            rc = rc * (2.0 - den * rc)
            return (pq.astype(f32) * rc).astype(bf16)

        def stage_b(s, c, pqn):
            cs = slice(c * CW2, (c + 1) * CW2)
            h_v[s, :, cs] = x_v[pl.ds(r0 + s * SB2, SB2), cs].astype(f32) + _dot(pqn, m_v[:, cs])

        def stage_c(s, c):
            h = h_v[s, c * RC:(c + 1) * RC, :]
            ln2 = _ln(h)
            rows = pl.ds(r0 + s * SB2 + c * RC, RC)
            out_v[rows, :] = (h + ln2).astype(bf16)
            ln2 = ln2.astype(bf16)
            ln2_v[rows, :] = ln2
            r_v[i * ns + s, c] = _dot_nt(wr, ln2)[0:8, :]

        def stage_r(s):
            o_copy(i * ns + s).start()

        pqn = {}
        for t in range(ns + 3):
            a = []
            for c in range(NC2):
                for st in ORD:
                    if st == 'b' and 0 <= t - 1 < ns:
                        stage_b(t - 1, c, pqn[t - 1])
                    if st == 'a' and t < ns:
                        a += [stage_a(t, g) for g in range(c * G // NC2, (c + 1) * G // NC2)]
                    if st == 'c' and 0 <= t - 2 < ns:
                        stage_c(t - 2, c)
                if c == RP and 0 <= t - 3 < ns:
                    stage_r(t - 3)
            if a:
                pqn[t] = jnp.concatenate(a, axis=1)

    jax.lax.fori_loop(0, NB2, p2, None)

    NS = S // SB2
    RC = SB2 // NC2 // CS
    r = r_v[...].reshape(S // RC, 8, RC)
    ids = (jax.lax.broadcasted_iota(jnp.int32, r.shape, 0) * RC
           + jax.lax.broadcasted_iota(jnp.int32, r.shape, 2))
    BIG = 1 << 20

    def red(op, a):
        return op(op(op(a, axis=0), axis=1, keepdims=True), axis=0, keepdims=True)

    m1 = red(jnp.max, r)
    i1 = red(jnp.min, jnp.where(r == m1, ids, BIG))
    r2 = jnp.where(ids == i1, -jnp.inf, r)
    m2 = red(jnp.max, r2)
    i2 = red(jnp.min, jnp.where((r2 == m2) & (ids != i1), ids, BIG))
    idx = [jnp.minimum(i1[0, 0], S - 1), jnp.minimum(i2[0, 0], S - 1)]
    gate = [jax.nn.sigmoid(m1), jax.nn.sigmoid(m2)]

    rows16 = jax.lax.broadcasted_iota(jnp.int32, (16, D), 0)
    xs = jnp.zeros((16, D), f32)
    bases = []
    for c in range(2):
        base = pl.multiple_of((idx[c] // 16) * 16, 16)
        bases.append(base)
        t = ln2_v[pl.ds(base, 16), :].astype(f32)
        row = jnp.sum(jnp.where(rows16 == idx[c] % 16, t, 0.0), axis=0, keepdims=True)
        xs = jnp.where(rows16 == c, row, xs)
    xs = xs.astype(bf16)
    c_wg.wait()
    c_wu.wait()
    c_wd.wait()
    for i in range(NS):
        o_copy(i).wait()
    FC = 512
    acts = []
    for f in range(0, F, FC):
        acts.append((jax.nn.silu(_dot(xs, wg_v[:, f:f + FC])) * _dot(xs, wu_v[:, f:f + FC])).astype(bf16))
    ys = [sum(_dot(acts[j], wd_v[j * FC:(j + 1) * FC, n:n + NW]) for j in range(F // FC)) for n in range(0, D, NW)]
    y = jnp.concatenate(ys, axis=1)
    for c in range(2):
        t = out_v[pl.ds(bases[c], 16), :].astype(f32)
        t = jnp.where(rows16 == idx[c] % 16, t + y[c:c + 1, :] * gate[c], t)
        out_v[pl.ds(bases[c], 16), :] = t.astype(bf16)

    def p_copy(c):
        return pltpu.make_async_copy(out_v.at[pl.ds(bases[c], 16)], out_hbm.at[pl.ds(bases[c], 16)], psem.at[c])

    p_copy(0).start()

    @pl.when(bases[0] != bases[1])
    def _():
        p_copy(1).start()
        p_copy(1).wait()

    p_copy(0).wait()


@jax.jit
def pallas_sequential_preLN__linear_attn_block__moe_arch_mod__prompt_kernel(
        A_x, A_wqkv, A_wo, B_x, B_w_r, B_w_gate, B_w_up, B_w_down):
    any_spec = pl.BlockSpec(memory_space=pl.ANY)
    V = pltpu.VMEM
    out = pl.pallas_call(
        _kernel,
        in_specs=[any_spec, any_spec, any_spec, pl.BlockSpec(memory_space=pltpu.VMEM), any_spec, any_spec, any_spec],
        out_specs=any_spec,
        out_shape=jax.ShapeDtypeStruct((S, D), bf16),
        scratch_shapes=[
            V((S, D), bf16), V((D, D), bf16), V((D, D), bf16), V((D, D), bf16), V((D, D), bf16), V((D, D), bf16),
            V((D, F), bf16), V((D, F), bf16), V((F, D), bf16),
            V((S, D), bf16), V((S, D), bf16), V((S, D), bf16),
            V((D, D), bf16), V((D, 128), bf16), V((D, 128), f32), V((D, 128), f32),
            V((HD, D), bf16), V((S // SB2, NC2 * CS, 8, SB2 // NC2 // CS), f32), V((TM2 // SB2, SB2, D), f32),
            pltpu.SemaphoreType.DMA((NB,)), pltpu.SemaphoreType.DMA((6 + NC,)),
            pltpu.SemaphoreType.DMA((S // SB2,)), pltpu.SemaphoreType.DMA((2,)),
        ],
        compiler_params=pltpu.CompilerParams(vmem_limit_bytes=100 * 1024 * 1024),
    )(A_x.reshape(S, D), A_wqkv, A_wo, B_w_r, B_w_gate, B_w_up, B_w_down)
    return out.reshape(1, S, D)
```
